```python
import os as _os
_os.environ.setdefault("JAX_PLATFORMS", "cpu")
import jax
import jax.numpy as jnp

def _softmax(x, axis=-1):
    return jax.nn.softmax(x, axis=axis)
def _gelu(x):
    return jax.nn.gelu(x, approximate=True)
def _silu(x):
    return jax.nn.silu(x)
def _sigmoid(x):
    return jax.nn.sigmoid(x)
def _layernorm(x, axis=-1, eps=1e-5):
    m = jnp.mean(x, axis=axis, keepdims=True)
    v = jnp.var(x, axis=axis, keepdims=True)
    return (x - m) / jnp.sqrt(v + eps)
def _scatter_add(tgt, idx, src, axis=0):
    return tgt.at[idx].add(src)
def _segment_sum(src, seg, n):
    return jax.ops.segment_sum(src, seg, n)
class _Rng:
    def __init__(self, key):
        self._k = key
    def _next(self):
        self._k, sub = jax.random.split(self._k)
        return sub
    def normal(self, shape):
        return jax.random.normal(self._next(), shape, dtype=jnp.bfloat16)
    def randint(self, lo, hi, shape):
        return jax.random.randint(self._next(), shape, lo, hi, dtype=jnp.int32)
    def uniform(self, shape, lo=0.0, hi=1.0):
        return jax.random.uniform(self._next(), shape, jnp.bfloat16, lo, hi)
    def permutation(self, n):
        return jax.random.permutation(self._next(), n)


kernel_name = 'gated_mix__ssm_conv_s5__glu_gated_geglu__prompt'

def setup_inputs():
    _rng = _Rng(jax.random.key(int.from_bytes(__import__("os").urandom(4), "little")))
    _w = (lambda a: (lambda t: t.astype(jnp.bfloat16) if jnp.issubdtype(t.dtype, jnp.floating) else t)(jnp.asarray(a)))
    def _A_setup():
        B, S, D = 1, 2048, 1024
        P = D
        Lambda_re = -0.5 * jnp.exp((lambda *s: _rng.normal(s) * 0.4)(P))
        Lambda_im = (lambda *s: _rng.normal(s) * 0.4)(P) * 1.0
        B_re = (lambda *s: _rng.normal(s) * 0.4)(P, D) * (D ** -0.5)
        B_im = (lambda *s: _rng.normal(s) * 0.4)(P, D) * (D ** -0.5)
        C_re = (lambda *s: _rng.normal(s) * 0.4)(D, P) * (P ** -0.5)
        C_im = (lambda *s: _rng.normal(s) * 0.4)(D, P) * (P ** -0.5)
        log_dt = (lambda *s: _rng.normal(s) * 0.4)(P) * 0.3 - 2.0
        Dskip = (lambda *s: _rng.normal(s) * 0.4)(D)
        return {
            "x": _w((lambda *s: _rng.normal(s) * 0.05)(B, S, D)),
            "Lambda_re": _w(Lambda_re),
            "Lambda_im": _w(Lambda_im),
            "B_re": _w(B_re),
            "B_im": _w(B_im),
            "C_re": _w(C_re),
            "C_im": _w(C_im),
            "log_dt": _w(log_dt),
            "Dskip": _w(Dskip),
        }
    _A_in = _A_setup()

    def _B_setup():
        B, S, Dm, Df = 1, 2048, 1024, 3584
        return {
            "x": _w((lambda *s: _rng.normal(s) * 0.05)(B, S, Dm)),
            "w_gate": _w((lambda *s: _rng.normal(s) * 1.6)(Dm, Df) * (Dm ** -0.5)),
            "w_up": _w((lambda *s: _rng.normal(s) * 1.6)(Dm, Df) * (Dm ** -0.5)),
            "w_down": _w((lambda *s: _rng.normal(s) * 1.6)(Df, Dm) * (Df ** -0.5)),
        }
    _B_in = _B_setup()

    return {
        "A_x": _A_in["x"],
        "A_Lambda_re": _A_in["Lambda_re"],
        "A_Lambda_im": _A_in["Lambda_im"],
        "A_B_re": _A_in["B_re"],
        "A_B_im": _A_in["B_im"],
        "A_C_re": _A_in["C_re"],
        "A_C_im": _A_in["C_im"],
        "A_log_dt": _A_in["log_dt"],
        "A_Dskip": _A_in["Dskip"],
        "B_x": _B_in["x"],
        "B_w_gate": _B_in["w_gate"],
        "B_w_up": _B_in["w_up"],
        "B_w_down": _B_in["w_down"],
        "gate_w": _w((lambda *s: _rng.normal(s) * 0.05)(1024) * 16.0),
    }

def reference(A_x, A_Lambda_re, A_Lambda_im, A_B_re, A_B_im, A_C_re, A_C_im, A_log_dt, A_Dskip, B_x, B_w_gate, B_w_up, B_w_down, gate_w):
    def _A_ref(x, Lambda_re, Lambda_im, B_re, B_im, C_re, C_im, log_dt, Dskip):
        Bsz, L, H = x.shape
        Lam = Lambda_re + 1j * Lambda_im
        Bmat = B_re + 1j * B_im
        Cmat = C_re + 1j * C_im
        dt = jnp.exp(log_dt)
        Lam_bar = jnp.exp(dt * Lam)
        B_bar = ((Lam_bar - 1.0) / Lam)[:, None] * Bmat
        Bu = jnp.einsum("bld,pd->blp", x + 0j, B_bar)
        h = jnp.zeros_like(Bu[:, 0, :])
        hs = []
        for t in range(L):
            h = Lam_bar[None, :] * h + Bu[:, t, :]
            hs.append(h)
        hseq = jnp.stack(hs, 1)
        y = 2.0 * jnp.einsum("blp,dp->bld", hseq, Cmat).real + x * Dskip[None, None, :]
        return y

    def _B_ref(x, w_gate, w_up, w_down):
        g = jnp.einsum("bsd,df->bsf", x, w_gate)
        u = jnp.einsum("bsd,df->bsf", x, w_up)
        h = _gelu(g) * u
        return jnp.einsum("bsf,fd->bsd", h, w_down)

    x = A_x
    g = _sigmoid((x * gate_w).sum(-1, keepdims=True))
    a = _A_ref(x, A_Lambda_re, A_Lambda_im, A_B_re, A_B_im, A_C_re, A_C_im, A_log_dt, A_Dskip)
    b = _B_ref(x, B_w_gate, B_w_up, B_w_down)
    return g * a + (1 - g) * b
```

```python
import jax
import jax.numpy as jnp
from jax import lax
import jax.experimental.pallas as pl
import jax.experimental.pallas.tpu as pltpu

T = 2048
D = 1024
P = 1024
F = 3584
TM = 512
NTL = T // TM
RQ = TM // 4
PR = T // 4
FC = 256
NC = F // FC
S1 = 9
SPI = -(-T // NC)
ZR = -(-(SPI * NC * S1) // 8) * 8
CSU = 5
GROUPS = ((0,), (1, 2), (3, 4, 5), (6, 7))
f32, bf16, u32 = jnp.float32, jnp.bfloat16, jnp.uint32
NT = (((1,), (1,)), ((), ()))


def _quads(X):
    n = len(X) // 2
    q = lambda r, c: [row[c * n:(c + 1) * n] for row in X[r * n:(r + 1) * n]]
    return q(0, 0), q(0, 1), q(1, 0), q(1, 1)


def _add(X, Y):
    return [[a + b for a, b in zip(rx, ry)] for rx, ry in zip(X, Y)]


def _sub(X, Y):
    return [[a - b for a, b in zip(rx, ry)] for rx, ry in zip(X, Y)]


A_TERMS = (((1, 0), (1, 3)), ((1, 2), (1, 3)), ((1, 0),), ((1, 3),),
           ((1, 0), (1, 1)), ((1, 2), (-1, 0)), ((1, 1), (-1, 3)))
B_TERMS = (((1, 0), (1, 3)), ((1, 0),), ((1, 1), (-1, 3)), ((1, 2), (-1, 0)),
           ((1, 3),), ((1, 0), (1, 1)), ((1, 2), (1, 3)))


def _operand(terms, quad):
    X = quad(terms[0][1])
    for s, q in terms[1:]:
        X = _add(X, quad(q)) if s > 0 else _sub(X, quad(q))
    return X


def _leaves(terms, X):
    if len(X) == 1:
        return [X[0][0]]
    Q = _quads(X)
    return [lf for t in terms for lf in _leaves(terms, _operand(t, lambda q: Q[q]))]


def _one_leaf(terms, get, level, k):
    def expand(lv, kk):
        if lv == 0:
            return [(1, 0, 0)]
        m, h = 7 ** (lv - 1), 2 ** (lv - 1)
        return [(s * s2, r + (q // 2) * h, c + (q % 2) * h)
                for s, q in terms[kk // m] for s2, r, c in expand(lv - 1, kk % m)]
    tt = sorted(expand(level, k), key=lambda t: -t[0])
    acc = get(tt[0][1], tt[0][2])
    for s, r, c in tt[1:]:
        acc = acc + get(r, c) if s > 0 else acc - get(r, c)
    return acc


def _combine(get, level, done, base=0):
    if level == 0:
        done(0, 0, get(base))
        return
    n, h = 7 ** (level - 1), 2 ** (level - 1)

    def m(i):
        out = [[None] * h for _ in range(h)]

        def keep(r, c, v):
            out[r][c] = v
        _combine(get, level - 1, keep, base + i * n)
        return out

    def fin(q, X):
        for r in range(h):
            for c in range(h):
                done((q // 2) * h + r, (q % 2) * h + c, X[r][c])
    m1 = m(0); m4 = m(3); m5 = m(4)
    fin(0, _add(_sub(_add(m1, m4), m5), m(6)))
    m3 = m(2); fin(1, _add(m3, m5)); t = _add(m1, m3)
    m2 = m(1); fin(2, _add(m2, m4)); t = _sub(t, m2)
    fin(3, _add(t, m(5)))


def _mo(v, m):
    return v if isinstance(v, int) else pl.multiple_of(v, m)


def _dot(a, b):
    return jnp.dot(a, b, preferred_element_type=f32)


def _dot_nt(a, b):
    return lax.dot_general(a, b, NT, preferred_element_type=f32)


def _token(v):
    u = pltpu.bitcast(v[0:8, 0:128], u32)
    return pltpu.bitcast((u >> 31) & ((~u) >> 31), f32)


class _Jobs:
    def __init__(self, jobs=(), pace=True):
        self.q = list(jobs)
        self.pace = pace

    def spread(self, slots):
        total = len(self.q)
        st = [0, 0]

        def tick(v):
            st[0] += 1
            want = min(total, -(-total * st[0] // slots))
            if st[1] < want:
                tz = _token(v) if self.pace else None
                while st[1] < want:
                    self.q.pop(0)(tz)
                    st[1] += 1
        return tick

    def flush(self):
        while self.q:
            self.q.pop(0)(None)


def _kernel(x_hbm, lre_hbm, lim_hbm, ldt_hbm, dsk_hbm, gw_hbm, bre_hbm, bim_hbm, cre_hbm, cim_hbm,
            wg_hbm, wu_hbm, wd_hbm, o_hbm,
            xb, vec, bb, cc, wg, wu, wd, xa, us, ds, cs, acc, zre, zim, cst, rows, gsc,
            xsem, bsem, fsem, vsem, osem):
    def x_copy(t):
        rs = pl.ds(_mo(t * TM, TM), TM)
        return pltpu.make_async_copy(x_hbm.at[rs], xb.at[rs], xsem.at[t])

    def b_copies(j):
        rs = pl.ds(_mo(j * 128, 128), 128)
        rs2 = pl.ds(_mo(P + j * 128, 128), 128)
        return (pltpu.make_async_copy(bre_hbm.at[rs], bb.at[rs], bsem.at[j, 0]),
                pltpu.make_async_copy(bim_hbm.at[rs], bb.at[rs2], bsem.at[j, 1]))

    def up_copies(c):
        csl = pl.ds(_mo(c * FC, FC), FC)
        return (pltpu.make_async_copy(wg_hbm.at[:, csl], wg.at[c], fsem.at[c, 0]),
                pltpu.make_async_copy(wu_hbm.at[:, csl], wu.at[c], fsem.at[c, 1]))

    def down_copy(c):
        csl = pl.ds(_mo(c * FC, FC), FC)
        return pltpu.make_async_copy(wd_hbm.at[csl], wd.at[c], fsem.at[c, 2])

    vec_copies = [pltpu.make_async_copy(r, vec.at[k], vsem.at[k])
                  for k, r in enumerate((lre_hbm, lim_hbm, ldt_hbm, dsk_hbm, gw_hbm))]
    c_copies = [pltpu.make_async_copy(cre_hbm, cc.at[:, pl.ds(0, P)], vsem.at[5]),
                pltpu.make_async_copy(cim_hbm, cc.at[:, pl.ds(P, P)], vsem.at[6])]

    def start_all(cps):
        for cp in cps:
            cp.start()

    def wait_all(cps):
        for cp in cps:
            cp.wait()

    start_all([x_copy(0), *b_copies(0), *vec_copies])

    def start_rest(i, _):
        @pl.when(i < 7)
        def _():
            start_all(b_copies(i + 1))

        @pl.when(i == 7)
        def _():
            start_all([x_copy(1), *up_copies(0)])

        @pl.when(i == 8)
        def _():
            start_all([x_copy(2), x_copy(3), down_copy(0)])

        @pl.when(i == 9)
        def _():
            start_all([*up_copies(1), down_copy(1), *c_copies])
    lax.fori_loop(0, 10, start_rest, None)

    def setup_consts():
        lre = vec[0].astype(f32)
        lim = vec[1].astype(f32)
        dt = jnp.exp(vec[2].astype(f32))
        mag = jnp.exp(dt * lre)
        are = mag * jnp.cos(dt * lim)
        aim = mag * jnp.sin(dt * lim)
        den = lre * lre + lim * lim
        cr = 2.0 * ((are - 1.0) * lre + aim * lim) / den
        ci = 2.0 * (aim * lre - (are - 1.0) * lim) / den
        cst[0] = are
        cst[1] = aim
        dsk = vec[3].astype(f32)
        gw = vec[4].astype(f32)
        for j in range(8):
            for k, v in enumerate((dsk, gw, cr, ci)):
                rows[k, :, j * 128:(j + 1) * 128] = jnp.broadcast_to(v[j:j + 1, :], (8, 128))
        npad = ZR - T * S1
        zre[pl.ds(T * S1, npad), :] = jnp.zeros((npad, 128), f32)
        zim[pl.ds(T * S1, npad), :] = jnp.zeros((npad, 128), f32)

    def unit(terms, blk0, dst, level, r_dst, l):
        nk = 7 ** level

        def paced(tz):
            if tz is None:
                return blk0
            tz2 = jnp.concatenate([tz, tz], axis=0)
            return lambda r, c: blk0(r, c) + tz2

        def store(grp, g):
            pk = pltpu.bitcast(jnp.concatenate(grp, axis=1).astype(bf16), u32)
            dst[pl.ds(_mo(r_dst // 2, 8), 8), pl.ds(_mo((l * nk + 7 * g) * 128, 128), 7 * 128)] = pk

        if level == 1:
            def job(tz):
                blk = paced(tz)
                store(_leaves(terms, [[blk(r, c) for c in range(2)] for r in range(2)]), 0)
            return [job]

        def sub(g):
            def job(tz):
                blk = paced(tz)
                quad = lambda q: [[blk((q // 2) * 2 + r, (q % 2) * 2 + c) for c in range(2)] for r in range(2)]
                store(_leaves(terms, _operand(terms[g], quad)), g)
            return job
        return [sub(g) for g in range(7)]

    def leaf(buf, k, nk, nl):
        parts = [buf[:, pl.ds((l * nk + k) * 128, 128)] for l in range(nl)]
        return pltpu.bitcast(parts[0] if nl == 1 else jnp.concatenate(parts, axis=1), bf16)

    def xa_jobs(t, i0, r_dst):
        out = []
        for l in range(2):
            blk = lambda r, c, l=l: xb[pl.ds(_mo(t * TM + r * RQ + i0, 16), 16),
                                       pl.ds(c * 256 + l * 128, 128)].astype(f32)
            out += unit(A_TERMS, blk, xa, 2, r_dst, l)
        return out

    def us_jobs(c, i0):
        blk = lambda r, s: (wg if s < 2 else wu)[c, pl.ds(_mo(r * 256 + i0, 16), 16),
                                                 pl.ds((s % 2) * 128, 128)].astype(f32)
        return unit(B_TERMS, blk, us, 2, i0, 0)

    def ds_jobs(c):
        out = []
        for i0 in range(0, 128, 16):
            for l in range(4):
                blk = lambda r, s, i0=i0, l=l: wd[c, pl.ds(r * 128 + i0, 16),
                                                  pl.ds(s * 512 + l * 128, 128)].astype(f32)
                out += unit(B_TERMS, blk, ds, 1, i0, l)
        return out

    def cs_jobs(u):
        i0 = _mo((u // 4) * 16, 16)
        l = u % 4
        blk = lambda r, s: cc[pl.ds(_mo(s * 256 + i0, 16), 16),
                              pl.ds(_mo(r * 512 + l * 128, 128), 128)].astype(f32)
        return unit(B_TERMS, blk, cs, 2, i0, l)

    def gate_job(r0, n):
        def job(tz):
            rs = pl.ds(_mo(r0, 8), n)
            gw = rows[1, 0:1, :]
            if tz is not None:
                gw = gw + jnp.concatenate([tz[0:1]] * 8, axis=1)
            gl = jnp.sum(xb[rs, :].astype(f32) * gw, axis=-1, keepdims=True)
            gsc[rs, :] = jnp.broadcast_to(jax.nn.sigmoid(gl), (n, 128))
            acc[rs, :] = jnp.zeros((n, D), f32)
        return job

    def bu_tile(r0, js, tick):
        for j in js:
            ure = _dot_nt(xb[pl.ds(r0, TM), :], bb[pl.ds(j * 128, 128), :])
            tick(ure)
            uim = _dot_nt(xb[pl.ds(r0, TM), :], bb[pl.ds(P + j * 128, 128), :])
            tick(uim)
            cr = rows[2, 0:1, j * 128:(j + 1) * 128]
            ci = rows[3, 0:1, j * 128:(j + 1) * 128]
            zre[pl.ds(r0 * S1 + j, TM, stride=S1), :] = cr * ure - ci * uim
            zim[pl.ds(r0 * S1 + j, TM, stride=S1), :] = -(cr * uim + ci * ure)

    for gi, grp in enumerate(GROUPS):
        if gi == 0:
            x_copy(0).wait()
            wait_all(vec_copies)
        for j in grp:
            wait_all(b_copies(j))
        if gi == 0:
            setup_consts()
        bu_tile(0, grp, lambda v: None)
    wait_all(up_copies(0))

    def p1_body(t, _):
        x_copy(t).wait()
        fl = _Jobs()
        for i in range(8):
            fl.q += xa_jobs(t, 16 * i, t * RQ + 16 * i)
            if i % 3 == 0:
                i0 = jnp.minimum(48 * (t - 1) + 16 * (i // 3), RQ - 16)
                fl.q += xa_jobs(0, i0, i0)
            if i % 4 != 3:
                fl.q += us_jobs(0, jnp.minimum(96 * (t - 1) + 16 * (i - i // 4), 240))
            if i % 2 == 1:
                fl.q.append(gate_job(t * TM + (i // 2) * 128, 128))
        fl.q.append(gate_job(jnp.minimum(176 * (t - 1), TM - 176), 176))
        bu_tile(_mo(t * TM, TM), range(8), fl.spread(14))
        fl.flush()
    lax.fori_loop(1, NTL, p1_body, None)
    wait_all(c_copies)

    def p2_body(c, carry):
        st = list(carry)

        @pl.when(c + 2 < NC)
        def _():
            start_all([*up_copies(c + 2), down_copy(c + 2)])
        down_copy(c).wait()

        @pl.when(c + 1 < NC)
        def _():
            wait_all(up_copies(c + 1))
        are = cst[0]
        aim = cst[1]
        base = c * (SPI * S1)

        def scan_job(k):
            def job(tz):
                sl = pl.ds(base + k * S1, 8)
                hr, hn = st
                if tz is not None:
                    hr = hr + tz
                nr = (are * hr + zre[sl, :]) + aim * hn
                nn = (are * hn + zim[sl, :]) - aim * hr
                zre[sl, :] = nr
                zim[sl, :] = nn
                st[0], st[1] = nr, nn
            return job
        fs = _Jobs([scan_job(k) for k in range(SPI)])
        fd = _Jobs(ds_jobs(c))
        tick_s = fs.spread(49 + 5)
        tick_d = fd.spread(44)

        def up_get(k):
            v = _dot(leaf(xa, k, 49, 2), leaf(us, k, 49, 1))
            tick_s(v)
            tick_d(v)
            return v
        blocks, H = {}, {}

        def up_done(q, s, v):
            blocks[(q, s)] = v
            if (q, s ^ 2) in blocks:
                H[(q, s % 2)] = jax.nn.gelu(blocks[(q, s % 2)], approximate=True) * blocks[(q, s % 2 + 2)]
        _combine(up_get, 2, up_done)
        fd.flush()
        cn = jnp.minimum(c + 1, NC - 1)
        fu = _Jobs([j for i0 in range(0, 256, 16) for j in us_jobs(cn, i0)]
                   + [j for i in range(CSU) for j in cs_jobs(jnp.minimum(CSU * c + i, 63))], pace=False)
        tick_u = fu.spread(6)
        Aq = {}

        def getq(r, s):
            if (r, s) not in Aq:
                Aq[(r, s)] = jnp.concatenate([H[(2 * r, s)], H[(2 * r + 1, s)]], axis=0)
            return Aq[(r, s)]

        def down_get(k):
            a = _one_leaf(A_TERMS, getq, 1, k)
            a2 = jnp.concatenate([a[:PR], a[PR:]], axis=1).astype(bf16)
            a = jnp.concatenate([a2[:, :128], a2[:, 128:]], axis=0)
            v = _dot(a, leaf(ds, k, 7, 4))
            tick_u(v)
            tick_s(v)
            return v

        def down_done(r, s, v):
            acc[pl.ds(r * (T // 2), T // 2), pl.ds(s * (D // 2), D // 2)] += v
        _combine(down_get, 1, down_done)
        fu.flush()
        fs.flush()
        return st[0], st[1]
    z = jnp.zeros((8, 128), f32)
    lax.fori_loop(0, NC, p2_body, (z, z))

    def p3_body(t, _):
        def zblk(q, s):
            zz = zre if s < 2 else zim
            return jnp.concatenate([zz[pl.ds((t * TM + q * RQ) * S1 + (s % 2) * 4 + l, RQ, stride=S1), :]
                                    for l in range(4)], axis=1)

        def p3_get(k):
            return _dot_nt(_one_leaf(A_TERMS, zblk, 2, k).astype(bf16), leaf(cs, k, 49, 4))

        def p3_done(q, s, y):
            col = pl.ds(s * 256, 256)
            nat = pl.ds(_mo(t * TM + q * RQ, RQ), RQ)
            prm = pl.ds(_mo(q * PR + t * RQ, RQ), RQ)
            g = jnp.concatenate([gsc[nat, :]] * 2, axis=1)
            pre = g * (xb[nat, col].astype(f32) * rows[0, 0:1, s * 256:(s + 1) * 256]) + (1.0 - g) * acc[prm, col]
            acc[prm, col] = g * y + pre
            pltpu.make_async_copy(acc.at[prm, col], o_hbm.at[nat, col], osem.at[0]).start()
        _combine(p3_get, 2, p3_done)
    lax.fori_loop(0, NTL, p3_body, None)
    pltpu.make_async_copy(acc, o_hbm, osem.at[0]).wait()


@jax.jit
def pallas_gated_mix__ssm_conv_s5__glu_gated_geglu__prompt_kernel(
    A_x: jax.Array,
    A_Lambda_re: jax.Array,
    A_Lambda_im: jax.Array,
    A_B_re: jax.Array,
    A_B_im: jax.Array,
    A_C_re: jax.Array,
    A_C_im: jax.Array,
    A_log_dt: jax.Array,
    A_Dskip: jax.Array,
    B_x: jax.Array,
    B_w_gate: jax.Array,
    B_w_up: jax.Array,
    B_w_down: jax.Array,
    gate_w: jax.Array,
):
    del B_x
    v = lambda a: a.reshape(8, 128)
    V, S = pltpu.VMEM, pltpu.SemaphoreType.DMA
    out = pl.pallas_call(
        _kernel,
        in_specs=[pl.BlockSpec(memory_space=pl.ANY)] * 13,
        out_specs=pl.BlockSpec(memory_space=pl.ANY),
        out_shape=jax.ShapeDtypeStruct((T, D), f32),
        scratch_shapes=[
            V((T, D), bf16), V((5, 8, 128), bf16), V((2 * P, D), bf16), V((D, 2 * P), bf16),
            V((NC, D, FC), bf16), V((NC, D, FC), bf16), V((NC, FC, D), bf16),
            V((T // 8, 2 * 49 * 128), u32), V((128, 49 * 128), u32), V((64, 4 * 7 * 128), u32),
            V((128, 4 * 49 * 128), u32),
            V((T, D), f32), V((ZR, 128), f32), V((ZR, 128), f32),
            V((2, 8, 128), f32), V((4, 8, D), f32), V((T, 128), f32),
            S((NTL,)), S((8, 2)), S((NC, 3)), S((7,)), S((1,))],
        compiler_params=pltpu.CompilerParams(vmem_limit_bytes=124 * 1024 * 1024),
    )(A_x.reshape(T, D), v(A_Lambda_re), v(A_Lambda_im), v(A_log_dt), v(A_Dskip), v(gate_w),
      A_B_re, A_B_im, A_C_re, A_C_im, B_w_gate, B_w_up, B_w_down)
    return out.reshape(1, T, D)
```

```python
import jax
import jax.numpy as jnp
from jax import lax
import jax.experimental.pallas as pl
import jax.experimental.pallas.tpu as pltpu

T = 2048
D = 1024
P = 1024
F = 3584
TM = 512
NTL = T // TM
RQ = TM // 4
PR = T // 4
FC = 256
NC = F // FC
S1 = 9
SPI = -(-T // NC)
ZR = -(-(SPI * NC * S1) // 8) * 8
CSU = 5
GROUPS = ((4, 1), (5, 2, 6), (3, 7))
f32, bf16, u32 = jnp.float32, jnp.bfloat16, jnp.uint32
NT = (((1,), (1,)), ((), ()))
GK = 0.7978845608028654


def _quads(X):
    n = len(X) // 2
    q = lambda r, c: [row[c * n:(c + 1) * n] for row in X[r * n:(r + 1) * n]]
    return q(0, 0), q(0, 1), q(1, 0), q(1, 1)


def _add(X, Y):
    return [[a + b for a, b in zip(rx, ry)] for rx, ry in zip(X, Y)]


def _sub(X, Y):
    return [[a - b for a, b in zip(rx, ry)] for rx, ry in zip(X, Y)]


A_TERMS = (((1, 0), (1, 3)), ((1, 2), (1, 3)), ((1, 0),), ((1, 3),),
           ((1, 0), (1, 1)), ((1, 2), (-1, 0)), ((1, 1), (-1, 3)))
B_TERMS = (((1, 0), (1, 3)), ((1, 0),), ((1, 1), (-1, 3)), ((1, 2), (-1, 0)),
           ((1, 3),), ((1, 0), (1, 1)), ((1, 2), (1, 3)))


def _operand(terms, quad):
    X = quad(terms[0][1])
    for s, q in terms[1:]:
        X = _add(X, quad(q)) if s > 0 else _sub(X, quad(q))
    return X


def _leaves(terms, X):
    if len(X) == 1:
        return [X[0][0]]
    Q = _quads(X)
    return [lf for t in terms for lf in _leaves(terms, _operand(t, lambda q: Q[q]))]


def _one_leaf(terms, get, level, k):
    def expand(lv, kk):
        if lv == 0:
            return [(1, 0, 0)]
        m, h = 7 ** (lv - 1), 2 ** (lv - 1)
        return [(s * s2, r + (q // 2) * h, c + (q % 2) * h)
                for s, q in terms[kk // m] for s2, r, c in expand(lv - 1, kk % m)]
    tt = sorted(expand(level, k), key=lambda t: -t[0])
    acc = get(tt[0][1], tt[0][2])
    for s, r, c in tt[1:]:
        acc = acc + get(r, c) if s > 0 else acc - get(r, c)
    return acc


def _combine(get, level, done, base=0):
    if level == 0:
        done(0, 0, get(base))
        return
    n, h = 7 ** (level - 1), 2 ** (level - 1)

    def m(i):
        out = [[None] * h for _ in range(h)]

        def keep(r, c, v):
            out[r][c] = v
        _combine(get, level - 1, keep, base + i * n)
        return out

    def fin(q, X):
        for r in range(h):
            for c in range(h):
                done((q // 2) * h + r, (q % 2) * h + c, X[r][c])
    m1 = m(0); m4 = m(3); m5 = m(4)
    fin(0, _add(_sub(_add(m1, m4), m5), m(6)))
    m3 = m(2); fin(1, _add(m3, m5)); t = _add(m1, m3)
    m2 = m(1); fin(2, _add(m2, m4)); t = _sub(t, m2)
    fin(3, _add(t, m(5)))


def _mo(v, m):
    return v if isinstance(v, int) else pl.multiple_of(v, m)


def _dot(a, b):
    return jnp.dot(a, b, preferred_element_type=f32)


def _dot_nt(a, b):
    return lax.dot_general(a, b, NT, preferred_element_type=f32)


def _token(v):
    u = pltpu.bitcast(v[0:8, 0:128], u32)
    return pltpu.bitcast((u >> 31) & ((~u) >> 31), f32)


class _Jobs:
    def __init__(self, jobs=(), pace=True):
        self.q = list(jobs)
        self.pace = pace

    def spread(self, slots):
        total = len(self.q)
        st = [0, 0]

        def tick(v):
            st[0] += 1
            want = min(total, -(-total * st[0] // slots))
            if st[1] < want:
                tz = _token(v) if self.pace else None
                while st[1] < want:
                    self.q.pop(0)(tz)
                    st[1] += 1
        return tick

    def flush(self):
        while self.q:
            self.q.pop(0)(None)


def _kernel(x_hbm, lre_hbm, lim_hbm, ldt_hbm, dsk_hbm, gw_hbm, bre_hbm, bim_hbm, cre_hbm, cim_hbm,
            wg_hbm, wu_hbm, wd_hbm, o_hbm,
            xb, vec, bb, cc, wg, wu, wd, xa, us, ds, cs, bs, acc, zre, zim, cst, rows, gsc,
            xsem, bsem, fsem, vsem, osem):
    def x_copy(t):
        rs = pl.ds(_mo(t * TM, TM), TM)
        return pltpu.make_async_copy(x_hbm.at[rs], xb.at[rs], xsem.at[t])

    def b_copies(j):
        rs = pl.ds(_mo(j * 128, 128), 128)
        rs2 = pl.ds(_mo(P + j * 128, 128), 128)
        return (pltpu.make_async_copy(bre_hbm.at[rs], bb.at[rs], bsem.at[j, 0]),
                pltpu.make_async_copy(bim_hbm.at[rs], bb.at[rs2], bsem.at[j, 1]))

    def up_copies(c):
        csl = pl.ds(_mo(c * FC, FC), FC)
        return (pltpu.make_async_copy(wg_hbm.at[:, csl], wg.at[c], fsem.at[c, 0]),
                pltpu.make_async_copy(wu_hbm.at[:, csl], wu.at[c], fsem.at[c, 1]))

    def down_copy(c):
        csl = pl.ds(_mo(c * FC, FC), FC)
        return pltpu.make_async_copy(wd_hbm.at[csl], wd.at[c], fsem.at[c, 2])

    vec_copies = [pltpu.make_async_copy(r, vec.at[k], vsem.at[k])
                  for k, r in enumerate((lre_hbm, lim_hbm, ldt_hbm, dsk_hbm, gw_hbm))]
    c_copies = [pltpu.make_async_copy(cre_hbm, cc.at[:, pl.ds(0, P)], vsem.at[5]),
                pltpu.make_async_copy(cim_hbm, cc.at[:, pl.ds(P, P)], vsem.at[6])]

    def start_all(cps):
        for cp in cps:
            cp.start()

    def wait_all(cps):
        for cp in cps:
            cp.wait()

    x0_copies = [pltpu.make_async_copy(x_hbm.at[pl.ds(h * 256, 256)], xb.at[pl.ds(h * 256, 256)],
                                       xsem.at[NTL * h]) for h in range(2)]
    start_all([x0_copies[0], *b_copies(0)])

    def start_rest(i, _):
        @pl.when(i == 0)
        def _():
            start_all([x0_copies[1], *vec_copies])

        @pl.when((i >= 1) & (i < 8))
        def _():
            start_all(b_copies(jnp.clip(i // 2 + (i % 2) * 4, 0, 7)))

        @pl.when(i == 8)
        def _():
            start_all([x_copy(1), *up_copies(0)])

        @pl.when(i == 9)
        def _():
            start_all([x_copy(2), x_copy(3), down_copy(0)])

        @pl.when(i == 10)
        def _():
            start_all([*up_copies(1), down_copy(1), *c_copies])
    lax.fori_loop(0, 11, start_rest, None)

    def setup_consts():
        lre = vec[0].astype(f32)
        lim = vec[1].astype(f32)
        dt = jnp.exp(vec[2].astype(f32))
        mag = jnp.exp(dt * lre)
        are = mag * jnp.cos(dt * lim)
        aim = mag * jnp.sin(dt * lim)
        den = lre * lre + lim * lim
        cr = 2.0 * ((are - 1.0) * lre + aim * lim) / den
        ci = 2.0 * (aim * lre - (are - 1.0) * lim) / den
        cst[0] = are
        cst[1] = aim
        dsk = vec[3].astype(f32)
        gw = vec[4].astype(f32)
        for j in range(8):
            for k, v in enumerate((dsk, gw, cr, ci)):
                rows[k, :, j * 128:(j + 1) * 128] = jnp.broadcast_to(v[j:j + 1, :], (8, 128))
        npad = ZR - T * S1
        zre[pl.ds(T * S1, npad), :] = jnp.zeros((npad, 128), f32)
        zim[pl.ds(T * S1, npad), :] = jnp.zeros((npad, 128), f32)

    def unit(terms, blk0, dst, level, r_dst, l, whole=False):
        nk = 7 ** level

        def paced(tz):
            if tz is None:
                return blk0
            tz2 = jnp.concatenate([tz, tz], axis=0)
            return lambda r, c: blk0(r, c) + tz2

        def store(grp, g):
            pk = pltpu.bitcast(jnp.concatenate(grp, axis=1).astype(bf16), u32)
            dst[pl.ds(_mo(r_dst // 2, 8), 8), pl.ds(_mo((l * nk + 7 * g) * 128, 128), 7 * 128)] = pk

        if level == 1 or whole:
            def job(tz):
                blk = paced(tz)
                n = 2 ** level
                lv = _leaves(terms, [[blk(r, c) for c in range(n)] for r in range(n)])
                for g in range(nk // 7):
                    store(lv[7 * g:7 * g + 7], g)
            return [job]

        def sub(g):
            def job(tz):
                blk = paced(tz)
                quad = lambda q: [[blk((q // 2) * 2 + r, (q % 2) * 2 + c) for c in range(2)] for r in range(2)]
                store(_leaves(terms, _operand(terms[g], quad)), g)
            return job
        return [sub(g) for g in range(7)]

    def leaf(buf, k, nk, nl):
        parts = [buf[:, pl.ds((l * nk + k) * 128, 128)] for l in range(nl)]
        return pltpu.bitcast(parts[0] if nl == 1 else jnp.concatenate(parts, axis=1), bf16)

    def xa_jobs(t, i0, r_dst):
        out = []
        for l in range(2):
            blk = lambda r, c, l=l: xb[pl.ds(_mo(t * TM + r * RQ + i0, 16), 16),
                                       pl.ds(c * 256 + l * 128, 128)].astype(f32)
            out += unit(A_TERMS, blk, xa, 2, r_dst, l)
        return out

    def us_jobs(c, i0):
        blk = lambda r, s: (wg if s < 2 else wu)[c, pl.ds(_mo(r * 256 + i0, 16), 16),
                                                 pl.ds((s % 2) * 128, 128)].astype(f32)
        return unit(B_TERMS, blk, us, 2, i0, 0)

    def ds_jobs(c):
        out = []
        for i0 in range(0, 128, 16):
            for l in range(4):
                blk = lambda r, s, i0=i0, l=l: wd[c, pl.ds(r * 128 + i0, 16),
                                                  pl.ds(s * 512 + l * 128, 128)].astype(f32)
                out += unit(B_TERMS, blk, ds, 1, i0, l)
        return out

    def cs_jobs(u):
        i0 = _mo((u // 4) * 16, 16)
        l = u % 4
        blk = lambda r, s: cc[pl.ds(_mo(s * 256 + i0, 16), 16),
                              pl.ds(_mo(r * 512 + l * 128, 128), 128)].astype(f32)
        return unit(B_TERMS, blk, cs, 2, i0, l)

    def bs_jobs(b):
        out = []
        for i0 in range(b * 128, (b + 1) * 128, 16):
            for l in range(2):
                blk = lambda r, s, i0=i0, l=l: bb[pl.ds(s * 512 + i0, 16), pl.ds(r * 256 + l * 128, 128)].astype(f32)
                out += unit(B_TERMS, blk, bs, 2, i0, l, whole=True)
        return out

    def gate_job(r0, n):
        def job(tz):
            rs = pl.ds(_mo(r0, 8), n)
            gw = rows[1, 0:1, :]
            if tz is not None:
                gw = gw + jnp.concatenate([tz[0:1]] * 8, axis=1)
            gl = jnp.sum(xb[rs, :].astype(f32) * gw, axis=-1, keepdims=True)
            gsc[rs, :] = jnp.broadcast_to(jax.nn.sigmoid(gl), (n, 128))
            acc[rs, :] = jnp.zeros((n, D), f32)
        return job

    def bu_store(r0, n, j, ure, uim):
        cr = rows[2, 0:1, j * 128:(j + 1) * 128]
        ci = rows[3, 0:1, j * 128:(j + 1) * 128]
        zre[pl.ds(r0 * S1 + j, n, stride=S1), :] = cr * ure - ci * uim
        zim[pl.ds(r0 * S1 + j, n, stride=S1), :] = -(cr * uim + ci * ure)

    def bu_tile(r0, js, tick):
        for j in js:
            ure = _dot_nt(xb[pl.ds(r0, TM), :], bb[pl.ds(j * 128, 128), :])
            tick(ure)
            uim = _dot_nt(xb[pl.ds(r0, TM), :], bb[pl.ds(P + j * 128, 128), :])
            tick(uim)
            bu_store(r0, TM, j, ure, uim)

    x0_copies[0].wait()
    wait_all(b_copies(0))
    ua = [_dot_nt(xb[pl.ds(0, 256), :], bb[pl.ds(o, 128), :]) for o in (0, P)]
    x0_copies[1].wait()
    wait_all(vec_copies)
    setup_consts()
    ub = [_dot_nt(xb[pl.ds(256, 256), :], bb[pl.ds(o, 128), :]) for o in (0, P)]
    bu_store(0, 256, 0, *ua)
    bu_store(256, 256, 0, *ub)
    for grp, rb in zip(GROUPS, ((0,), (1, 2), (3,))):
        for j in grp:
            wait_all(b_copies(j))
        fb = _Jobs([j for b in rb for j in bs_jobs(b)], pace=False)
        bu_tile(0, grp, fb.spread(2 * len(grp) - 1))
        fb.flush()
    wait_all(up_copies(0))

    def p1_body(t, _):
        x_copy(t).wait()
        ORD = (0, 3, 4, 6, 2, 1, 5)
        xj = [xa_jobs(t, 16 * i, t * RQ + 16 * i) for i in range(8)]
        sel = lambda g: [u[7 * l + g] for u in xj for l in range(2)]
        fl = _Jobs(pace=True)
        for i in range(8):
            if i % 3 == 0:
                i0 = jnp.minimum(48 * (t - 1) + 16 * (i // 3), RQ - 16)
                fl.q += xa_jobs(0, i0, i0)
            if i % 4 != 3:
                fl.q += us_jobs(0, jnp.minimum(96 * (t - 1) + 16 * (i - i // 4), 240))
            if i % 2 == 1:
                fl.q.append(gate_job(t * TM + (i // 2) * 128, 128))
        fl.q.append(gate_job(jnp.minimum(176 * (t - 1), TM - 176), 176))
        tick_o = fl.spread(44)
        _Jobs(sel(ORD[0])).flush()
        cnt = [0, None, None]
        pr = pl.ds(_mo(t * (RQ // 2), 8), RQ // 2)

        def p1_get(k):
            n = cnt[0]; cnt[0] += 1
            if n % 7 == 0:
                if cnt[1] is not None: cnt[1].flush()
                cnt[1] = _Jobs(sel(ORD[n // 7 + 1]) if n < 42 else [], pace=True); cnt[2] = cnt[1].spread(5)
            a = jnp.concatenate([xa[pr, pl.ds((l * 49 + k) * 128, 128)] for l in range(2)], axis=1)
            v = _dot_nt(pltpu.bitcast(a, bf16), leaf(bs, k, 49, 2))
            cnt[2](v); tick_o(v)
            return v
        res = {}

        def p1_done(q, s, v):
            res[(q, s)] = v
            if s >= 2:
                for l in range(4):
                    bu_store(_mo(t * TM + q * RQ, RQ), RQ, (s - 2) * 4 + l,
                             res[(q, s - 2)][:, l * 128:(l + 1) * 128], v[:, l * 128:(l + 1) * 128])
        _combine(p1_get, 2, p1_done)
        fl.flush()
    lax.fori_loop(1, NTL, p1_body, None)
    wait_all(c_copies)

    def p2_body(c, carry):
        st = list(carry)

        @pl.when(c + 2 < NC)
        def _():
            start_all([*up_copies(c + 2), down_copy(c + 2)])
        down_copy(c).wait()

        @pl.when(c + 1 < NC)
        def _():
            wait_all(up_copies(c + 1))
        are = cst[0]
        aim = cst[1]
        base = c * (SPI * S1)

        def scan_job(k):
            def job(_):
                sl = pl.ds(base + k * S1, 8)
                hr, hn = st
                nr = (are * hr + zre[sl, :]) + aim * hn
                nn = (are * hn + zim[sl, :]) - aim * hr
                zre[sl, :] = nr
                zim[sl, :] = nn
                st[0], st[1] = nr, nn
            return job
        fs = _Jobs([scan_job(k) for k in range(SPI)], pace=False)
        fd = _Jobs(ds_jobs(c))
        tick_s = fs.spread(49 + 5)
        tick_d = fd.spread(44)

        def up_get(k):
            v = _dot(leaf(xa, k, 49, 2), leaf(us, k, 49, 1))
            tick_s(v)
            tick_d(v)
            return v
        blocks, H = {}, {}

        def up_done(q, s, v):
            blocks[(q, s)] = v
            if (q, s ^ 2) in blocks:
                g, u = blocks[(q, s % 2)], blocks[(q, s % 2 + 2)]
                H[(q, s % 2)] = (g * u) * (jnp.tanh(g * (g * g * (GK * 0.044715) + GK)) + 1.0)
        _combine(up_get, 2, up_done)
        fd.flush()
        cn = jnp.minimum(c + 1, NC - 1)
        fu = _Jobs([j for i0 in range(0, 256, 16) for j in us_jobs(cn, i0)]
                   + [j for i in range(CSU) for j in cs_jobs(jnp.minimum(CSU * c + i, 63))], pace=False)
        tick_u = fu.spread(6)
        Aq = {}

        def getq(r, s):
            if (r, s) not in Aq:
                Aq[(r, s)] = jnp.concatenate([H[(2 * r, s)], H[(2 * r + 1, s)]], axis=0)
            return Aq[(r, s)]

        def down_get(k):
            a = _one_leaf(A_TERMS, getq, 1, k)
            a2 = jnp.concatenate([a[:PR], a[PR:]], axis=1).astype(bf16)
            a = jnp.concatenate([a2[:, :128], a2[:, 128:]], axis=0)
            v = _dot(a, leaf(ds, k, 7, 4))
            tick_u(v)
            tick_s(v)
            return v

        def down_done(r, s, v):
            acc[pl.ds(r * (T // 2), T // 2), pl.ds(s * (D // 2), D // 2)] += v
        _combine(down_get, 1, down_done)
        fu.flush()
        fs.flush()
        return st[0], st[1]
    z = jnp.zeros((8, 128), f32)
    lax.fori_loop(0, NC, p2_body, (z, z))

    def p3_body(t, _):
        def zblk(q, s):
            zz = zre if s < 2 else zim
            return jnp.concatenate([zz[pl.ds((t * TM + q * RQ) * S1 + (s % 2) * 4 + l, RQ, stride=S1), :]
                                    for l in range(4)], axis=1)

        def p3_get(k):
            return _dot_nt(_one_leaf(A_TERMS, zblk, 2, k).astype(bf16), leaf(cs, k, 49, 4))

        def p3_done(q, s, y):
            col = pl.ds(s * 256, 256)
            nat = pl.ds(_mo(t * TM + q * RQ, RQ), RQ)
            prm = pl.ds(_mo(q * PR + t * RQ, RQ), RQ)
            g = jnp.concatenate([gsc[nat, :]] * 2, axis=1)
            pre = g * (xb[nat, col].astype(f32) * rows[0, 0:1, s * 256:(s + 1) * 256]) + (0.5 - 0.5 * g) * acc[prm, col]
            acc[prm, col] = g * y + pre
            pltpu.make_async_copy(acc.at[prm, col], o_hbm.at[nat, col], osem.at[0]).start()
        _combine(p3_get, 2, p3_done)
    lax.fori_loop(0, NTL, p3_body, None)
    pltpu.make_async_copy(acc, o_hbm, osem.at[0]).wait()


@jax.jit
def pallas_gated_mix__ssm_conv_s5__glu_gated_geglu__prompt_kernel(
    A_x: jax.Array,
    A_Lambda_re: jax.Array,
    A_Lambda_im: jax.Array,
    A_B_re: jax.Array,
    A_B_im: jax.Array,
    A_C_re: jax.Array,
    A_C_im: jax.Array,
    A_log_dt: jax.Array,
    A_Dskip: jax.Array,
    B_x: jax.Array,
    B_w_gate: jax.Array,
    B_w_up: jax.Array,
    B_w_down: jax.Array,
    gate_w: jax.Array,
):
    del B_x
    v = lambda a: a.reshape(8, 128)
    V, S = pltpu.VMEM, pltpu.SemaphoreType.DMA
    out = pl.pallas_call(
        _kernel,
        in_specs=[pl.BlockSpec(memory_space=pl.ANY)] * 13,
        out_specs=pl.BlockSpec(memory_space=pl.ANY),
        out_shape=jax.ShapeDtypeStruct((T, D), f32),
        scratch_shapes=[
            V((T, D), bf16), V((5, 8, 128), bf16), V((2 * P, D), bf16), V((D, 2 * P), bf16),
            V((NC, D, FC), bf16), V((NC, D, FC), bf16), V((NC, FC, D), bf16),
            V((T // 8, 2 * 49 * 128), u32), V((128, 49 * 128), u32), V((64, 4 * 7 * 128), u32),
            V((128, 4 * 49 * 128), u32), V((256, 2 * 49 * 128), u32),
            V((T, D), f32), V((ZR, 128), f32), V((ZR, 128), f32),
            V((2, 8, 128), f32), V((4, 8, D), f32), V((T, 128), f32),
            S((NTL + 1,)), S((8, 2)), S((NC, 3)), S((7,)), S((1,))],
        compiler_params=pltpu.CompilerParams(vmem_limit_bytes=124 * 1024 * 1024),
    )(A_x.reshape(T, D), v(A_Lambda_re), v(A_Lambda_im), v(A_log_dt), v(A_Dskip), v(gate_w),
      A_B_re, A_B_im, A_C_re, A_C_im, B_w_gate, B_w_up, B_w_down)
    return out.reshape(1, T, D)
```
